```python
import os as _os
_os.environ.setdefault("JAX_PLATFORMS", "cpu")
import jax
import jax.numpy as jnp

def _softmax(x, axis=-1):
    return jax.nn.softmax(x, axis=axis)
def _gelu(x):
    return jax.nn.gelu(x, approximate=True)
def _silu(x):
    return jax.nn.silu(x)
def _sigmoid(x):
    return jax.nn.sigmoid(x)
def _layernorm(x, axis=-1, eps=1e-5):
    m = jnp.mean(x, axis=axis, keepdims=True)
    v = jnp.var(x, axis=axis, keepdims=True)
    return (x - m) / jnp.sqrt(v + eps)
def _scatter_add(tgt, idx, src, axis=0):
    return tgt.at[idx].add(src)
def _segment_sum(src, seg, n):
    return jax.ops.segment_sum(src, seg, n)
class _Rng:
    def __init__(self, key):
        self._k = key
    def _next(self):
        self._k, sub = jax.random.split(self._k)
        return sub
    def normal(self, shape):
        return jax.random.normal(self._next(), shape, dtype=jnp.bfloat16)
    def randint(self, lo, hi, shape):
        return jax.random.randint(self._next(), shape, lo, hi, dtype=jnp.int32)
    def uniform(self, shape, lo=0.0, hi=1.0):
        return jax.random.uniform(self._next(), shape, jnp.bfloat16, lo, hi)
    def permutation(self, n):
        return jax.random.permutation(self._next(), n)


kernel_name = 'standalone__mha_softmax__near_ridge'

def setup_inputs():
    _rng = _Rng(jax.random.key(int.from_bytes(__import__("os").urandom(4), "little")))
    _w = (lambda a: (lambda t: t.astype(jnp.bfloat16) if jnp.issubdtype(t.dtype, jnp.floating) else t)(jnp.asarray(a)))
    B, H, Sq, Sk, D = 8, 32, 304, 2048, 128
    return {
        "q": _w((lambda *s: _rng.normal(s) * 0.4)(B, H, Sq, D)),
        "k": _w((lambda *s: _rng.normal(s) * 0.4)(B, H, Sk, D)),
        "v": _w((lambda *s: _rng.normal(s) * 0.05)(B, H, Sk, D)),
    }

def reference(q, k, v):
    scale = q.shape[-1] ** -0.5
    scores = jnp.einsum("bhqd,bhkd->bhqk", q, k) * scale
    p = _softmax(scores, axis=-1)
    return jnp.einsum("bhqk,bhkd->bhqd", p, v)
```

```python
import jax
import jax.numpy as jnp
from jax import lax
import jax.experimental.pallas as pl
import jax.experimental.pallas.tpu as pltpu

_LOG2E = 1.4426950408889634


def _load_bf16(ref):
    return pltpu.bitcast(ref.bitcast(jnp.uint32)[...], jnp.bfloat16)


def _make_kernel(G, n_out_pieces):
    def kernel(q_hbm, k_hbm, v_hbm, o_hbm, qb, kb, vb, ob, sq, sk, sv, so):
        NH, Sq, D = q_hbm.shape
        n_it = NH // G
        c = D ** -0.5 * _LOG2E
        GP = G // n_out_pieces

        def cp_q(h, j): return pltpu.make_async_copy(q_hbm.at[h], qb.at[j], sq.at[j])
        def cp_k(h, j): return pltpu.make_async_copy(k_hbm.at[h], kb.at[j], sk.at[j])
        def cp_v(h, j): return pltpu.make_async_copy(v_hbm.at[h], vb.at[j], sv.at[j])
        def cp_o(h0, p):
            return pltpu.make_async_copy(ob.at[pl.ds(p * GP, GP)], o_hbm.at[pl.ds(h0 + p * GP, GP)], so.at[p])

        for j in range(G):
            cp_q(j, j).start()
            cp_k(j, j).start()
            cp_v(j, j).start()

        def body(it, carry):
            h0 = it * G
            more = it + 1 < n_it
            for j in range(G):
                h = h0 + j
                cp_q(h, j).wait()
                cp_k(h, j).wait()
                q = (_load_bf16(qb.at[j]).astype(jnp.float32) * c).astype(jnp.bfloat16)
                s = lax.dot_general(q, _load_bf16(kb.at[j]), (((1,), (1,)), ((), ())),
                                    preferred_element_type=jnp.float32)

                @pl.when(more)
                def _(h=h, j=j):
                    cp_q(h + G, j).start()
                    cp_k(h + G, j).start()

                m = jnp.max(s, axis=-1, keepdims=True)
                p = jnp.exp2(s - m)
                l = jnp.sum(p, axis=-1, keepdims=True)
                cp_v(h, j).wait()
                o = jnp.dot(p.astype(jnp.bfloat16), _load_bf16(vb.at[j]), preferred_element_type=jnp.float32)

                @pl.when(more)
                def _(h=h, j=j):
                    cp_v(h + G, j).start()

                if j % GP == 0:
                    @pl.when(it > 0)
                    def _(j=j):
                        cp_o(h0 - G, j // GP).wait()

                r = pl.reciprocal(l, approx=True)
                r = r * (2.0 - l * r)
                ob[j] = (o * r).astype(ob.dtype)
                if j % GP == GP - 1:
                    cp_o(h0, j // GP).start()
            return carry

        lax.fori_loop(0, n_it, body, 0)
        for p in range(n_out_pieces):
            cp_o(NH - G, p).wait()

    return kernel


@jax.jit
def pallas_standalone__mha_softmax__near_ridge_kernel(q: jax.Array, k: jax.Array, v: jax.Array):
    B, H, Sq, D = q.shape
    Sk = k.shape[2]
    NH = B * H
    G = 16
    n_out_pieces = 4
    q3 = q.reshape(NH, Sq, D)
    k3 = k.reshape(NH, Sk, D)
    v3 = v.reshape(NH, Sk, D)
    o = pl.pallas_call(
        _make_kernel(G, n_out_pieces),
        grid=(1,),
        in_specs=[pl.BlockSpec(memory_space=pl.ANY)] * 3,
        out_specs=pl.BlockSpec(memory_space=pl.ANY),
        out_shape=jax.ShapeDtypeStruct(q3.shape, q.dtype),
        scratch_shapes=[
            pltpu.VMEM((G, Sq, D), q.dtype),
            pltpu.VMEM((G, Sk, D), k.dtype),
            pltpu.VMEM((G, Sk, D), v.dtype),
            pltpu.VMEM((G, Sq, D), q.dtype),
            pltpu.SemaphoreType.DMA((G,)),
            pltpu.SemaphoreType.DMA((G,)),
            pltpu.SemaphoreType.DMA((G,)),
            pltpu.SemaphoreType.DMA((n_out_pieces,)),
        ],
        compiler_params=pltpu.CompilerParams(
            dimension_semantics=("arbitrary",),
            vmem_limit_bytes=64 << 20,
            flags={"XLA_TPU_RESCHEDULE_DMA_DONES": True},
            disable_bounds_checks=True,
        ),
    )(q3, k3, v3)
    return o.reshape(q.shape)
```

```python
import jax
import jax.numpy as jnp
from jax import lax
import jax.experimental.pallas as pl
import jax.experimental.pallas.tpu as pltpu

_LOG2E = 1.4426950408889634
_GROUP = 16
_PREFETCH = 4
_OUT_PIECES = 4


def _attention_kernel(q_hbm, k_hbm, v_hbm, o_hbm,
                      q_buf, k_buf, v_buf, o_buf, q_sem, k_sem, v_sem, o_sem):
    n_heads, sq, d = q_hbm.shape
    sk = k_hbm.shape[1]
    g = q_buf.shape[0]
    n_groups = n_heads // g
    per_piece = g // _OUT_PIECES
    n_tiles = sk // 128
    c = d ** -0.5 * _LOG2E

    def copy_q(h, slot):
        return pltpu.make_async_copy(q_hbm.at[h], q_buf.at[slot], q_sem.at[slot])

    def copy_k(h, slot):
        return pltpu.make_async_copy(k_hbm.at[h], k_buf.at[slot], k_sem.at[slot])

    def copy_v(h, slot):
        return pltpu.make_async_copy(v_hbm.at[h], v_buf.at[slot], v_sem.at[slot])

    def copy_o(h0, piece):
        rows = pl.ds(piece * per_piece, per_piece)
        return pltpu.make_async_copy(
            o_buf.at[rows], o_hbm.at[pl.ds(h0 + piece * per_piece, per_piece)], o_sem.at[piece])

    def fetch(h, slot):
        copy_q(h, slot).start()
        copy_k(h, slot).start()
        copy_v(h, slot).start()

    for j in range(_PREFETCH):
        fetch(j, j)

    def group(it, carry):
        h0 = it * g
        zero = jnp.minimum(it, 0).astype(jnp.float32)
        prev_sum = None
        for j in range(g):
            h = h0 + j
            copy_q(h, j).wait()
            copy_k(h, j).wait()
            s = lax.dot_general(q_buf[j], k_buf[j], (((1,), (1,)), ((), ())),
                                preferred_element_type=jnp.float32)

            @pl.when(h + _PREFETCH < n_heads)
            def _(h=h, j=j):
                fetch(h + _PREFETCH, (j + _PREFETCH) % g)

            cvec = c if prev_sum is None else jnp.concatenate(
                [jnp.where(prev_sum >= 0.0, c, c + zero)] * n_tiles, axis=-1)

            m = jnp.max(s, axis=-1, keepdims=True)
            p = jnp.exp2((s - m) * cvec)
            lane_sum = p[:, 0:128]
            for t in range(1, n_tiles):
                lane_sum = lane_sum + p[:, t * 128:(t + 1) * 128]
            prev_sum = lane_sum

            copy_v(h, j).wait()
            o = jnp.dot(p.astype(jnp.bfloat16), v_buf[j], preferred_element_type=jnp.float32)
            l = jnp.sum(lane_sum, axis=-1, keepdims=True)

            if j % per_piece == 0:
                @pl.when(it > 0)
                def _(j=j):
                    copy_o(h0 - g, j // per_piece).wait()

            o_buf[j] = (o * pl.reciprocal(l, approx=True)).astype(o_buf.dtype)
            if j % per_piece == per_piece - 1:
                copy_o(h0, j // per_piece).start()
        return carry

    lax.fori_loop(0, n_groups, group, 0)
    for piece in range(_OUT_PIECES):
        copy_o(n_heads - g, piece).wait()


@jax.jit
def pallas_standalone__mha_softmax__near_ridge_kernel(q: jax.Array, k: jax.Array, v: jax.Array):
    b, h, sq, d = q.shape
    sk = k.shape[2]
    n_heads = b * h
    g = _GROUP
    out = pl.pallas_call(
        _attention_kernel,
        grid=(1,),
        in_specs=[pl.BlockSpec(memory_space=pl.ANY)] * 3,
        out_specs=pl.BlockSpec(memory_space=pl.ANY),
        out_shape=jax.ShapeDtypeStruct((n_heads, sq, d), q.dtype),
        scratch_shapes=[
            pltpu.VMEM((g, sq, d), q.dtype),
            pltpu.VMEM((g, sk, d), k.dtype),
            pltpu.VMEM((g, sk, d), v.dtype),
            pltpu.VMEM((g, sq, d), q.dtype),
            pltpu.SemaphoreType.DMA((g,)),
            pltpu.SemaphoreType.DMA((g,)),
            pltpu.SemaphoreType.DMA((g,)),
            pltpu.SemaphoreType.DMA((_OUT_PIECES,)),
        ],
        compiler_params=pltpu.CompilerParams(
            dimension_semantics=("arbitrary",),
            vmem_limit_bytes=64 << 20,
            flags={"XLA_TPU_RESCHEDULE_DMA_DONES": True},
            disable_bounds_checks=True,
            disable_semaphore_checks=True,
        ),
    )(q.reshape(n_heads, sq, d), k.reshape(n_heads, sk, d), v.reshape(n_heads, sk, d))
    return out.reshape(q.shape)
```

```python
import functools

import jax
import jax.numpy as jnp
from jax import lax
import jax.experimental.pallas as pl
import jax.experimental.pallas.tpu as pltpu

_LOG2E = 1.4426950408889634
_LANES = 128
_MAX_GROUP = 16
_MAX_PREFETCH = 4
_MAX_OUT_PIECES = 4


def _attention_kernel(q_hbm, k_hbm, v_hbm, o_hbm,
                      q_buf, k_buf, v_buf, o_buf, q_sem, k_sem, v_sem, o_sem,
                      *, prefetch, out_pieces):
    n_heads, _, d = q_hbm.shape
    sk = k_hbm.shape[1]
    group = q_buf.shape[0]
    per_piece = group // out_pieces
    n_tiles = sk // _LANES
    c = d ** -0.5 * _LOG2E

    def copy_q(h, slot):
        return pltpu.make_async_copy(q_hbm.at[h], q_buf.at[slot], q_sem.at[slot])

    def copy_k(h, slot):
        return pltpu.make_async_copy(k_hbm.at[h], k_buf.at[slot], k_sem.at[slot])

    def copy_v(h, slot):
        return pltpu.make_async_copy(v_hbm.at[h], v_buf.at[slot], v_sem.at[slot])

    def copy_o(h0, piece):
        first = piece * per_piece
        return pltpu.make_async_copy(o_buf.at[pl.ds(first, per_piece)],
                                     o_hbm.at[pl.ds(h0 + first, per_piece)],
                                     o_sem.at[piece])

    def fetch(h, slot):
        copy_q(h, slot).start()
        copy_k(h, slot).start()
        copy_v(h, slot).start()

    for j in range(prefetch):
        fetch(j, j)

    def head_group(it, carry):
        h0 = it * group
        zero = jnp.minimum(it, 0).astype(jnp.float32)
        prev_lane_sum = None
        for j in range(group):
            h = h0 + j
            copy_q(h, j).wait()
            copy_k(h, j).wait()
            s = lax.dot_general(q_buf[j], k_buf[j], (((1,), (1,)), ((), ())),
                                preferred_element_type=jnp.float32)

            @pl.when(h + prefetch < n_heads)
            def _(h=h, j=j):
                fetch(h + prefetch, (j + prefetch) % group)

            if prev_lane_sum is None:
                scale = c
            else:
                scale = jnp.concatenate(
                    [jnp.where(prev_lane_sum >= 0.0, c, c + zero)] * n_tiles, axis=-1)

            m = jnp.max(s, axis=-1, keepdims=True)
            p = jnp.exp2((s - m) * scale)
            lane_sum = p[:, :_LANES]
            for t in range(1, n_tiles):
                lane_sum = lane_sum + p[:, t * _LANES:(t + 1) * _LANES]
            prev_lane_sum = lane_sum

            copy_v(h, j).wait()
            o = jnp.dot(p.astype(v_buf.dtype), v_buf[j], preferred_element_type=jnp.float32)
            l = jnp.sum(lane_sum, axis=-1, keepdims=True)

            if j % per_piece == 0:
                @pl.when(it > 0)
                def _(j=j):
                    copy_o(h0 - group, j // per_piece).wait()

            o_buf[j] = (o * pl.reciprocal(l, approx=True)).astype(o_buf.dtype)
            if j % per_piece == per_piece - 1:
                copy_o(h0, j // per_piece).start()
        return carry

    lax.fori_loop(0, n_heads // group, head_group, 0)
    for piece in range(out_pieces):
        copy_o(n_heads - group, piece).wait()


@jax.jit
def pallas_standalone__mha_softmax__near_ridge_kernel(q: jax.Array, k: jax.Array, v: jax.Array):
    b, h, sq, d = q.shape
    sk = k.shape[2]
    n_heads = b * h
    group = _MAX_GROUP
    while n_heads % group:
        group //= 2
    assert group >= 2 and sk % _LANES == 0, (q.shape, k.shape)
    prefetch = min(_MAX_PREFETCH, group - 1)
    out_pieces = min(_MAX_OUT_PIECES, group)

    out = pl.pallas_call(
        functools.partial(_attention_kernel, prefetch=prefetch, out_pieces=out_pieces),
        grid=(1,),
        in_specs=[pl.BlockSpec(memory_space=pl.ANY)] * 3,
        out_specs=pl.BlockSpec(memory_space=pl.ANY),
        out_shape=jax.ShapeDtypeStruct((n_heads, sq, d), q.dtype),
        scratch_shapes=[
            pltpu.VMEM((group, sq, d), q.dtype),
            pltpu.VMEM((group, sk, d), k.dtype),
            pltpu.VMEM((group, sk, d), v.dtype),
            pltpu.VMEM((group, sq, d), q.dtype),
            pltpu.SemaphoreType.DMA((group,)),
            pltpu.SemaphoreType.DMA((group,)),
            pltpu.SemaphoreType.DMA((group,)),
            pltpu.SemaphoreType.DMA((out_pieces,)),
        ],
        compiler_params=pltpu.CompilerParams(
            dimension_semantics=("arbitrary",),
            vmem_limit_bytes=64 << 20,
            flags={"XLA_TPU_RESCHEDULE_DMA_DONES": True},
            disable_bounds_checks=True,
            disable_semaphore_checks=True,
        ),
    )(q.reshape(n_heads, sq, d), k.reshape(n_heads, sk, d), v.reshape(n_heads, sk, d))
    return out.reshape(q.shape)
```

```python
import functools

import jax
import jax.numpy as jnp
from jax import lax
import jax.experimental.pallas as pl
import jax.experimental.pallas.tpu as pltpu

_LOG2E = 1.4426950408889634
_LANES = 128
_MAX_GROUP = 23
_MAX_UNROLLED = 26
_MAX_PREFETCH = 4
_MAX_OUT_PIECES = 4


def _split_heads(n_heads):
    best = None
    for group in range(min(_MAX_GROUP, n_heads), 1, -1):
        rest = n_heads % group
        if group + rest > _MAX_UNROLLED:
            continue
        n_blocks = n_heads // group + (rest > 0)
        if best is None or n_blocks < best[0]:
            best = (n_blocks, group, rest)
    assert best is not None, n_heads
    return best[1:]


def _pieces(n, parts):
    sizes = [n // parts + (i < n % parts) for i in range(parts)]
    return [(sum(sizes[:i]), sizes[i]) for i in range(parts)]


def _attention_kernel(q_hbm, k_hbm, v_hbm, o_hbm,
                      q_buf, k_buf, v_buf, o_buf, o_rest_buf,
                      q_sem, k_sem, v_sem, o_sem, o_rest_sem,
                      *, rest, prefetch, pieces):
    n_heads, _, d = q_hbm.shape
    sk = k_hbm.shape[1]
    group = q_buf.shape[0]
    n_tiles = sk // _LANES
    n_main = n_heads - rest
    c = d ** -0.5 * _LOG2E
    piece_of_first = {start: i for i, (start, _) in enumerate(pieces)}
    piece_of_last = {start + size - 1: i for i, (start, size) in enumerate(pieces)}

    def copy_q(h, slot):
        return pltpu.make_async_copy(q_hbm.at[h], q_buf.at[slot], q_sem.at[slot])

    def copy_k(h, slot):
        return pltpu.make_async_copy(k_hbm.at[h], k_buf.at[slot], k_sem.at[slot])

    def copy_v(h, slot):
        return pltpu.make_async_copy(v_hbm.at[h], v_buf.at[slot], v_sem.at[slot])

    def copy_o(h0, piece):
        start, size = pieces[piece]
        return pltpu.make_async_copy(o_buf.at[pl.ds(start, size)],
                                     o_hbm.at[pl.ds(h0 + start, size)], o_sem.at[piece])

    def copy_o_rest():
        return pltpu.make_async_copy(o_rest_buf, o_hbm.at[pl.ds(n_main, rest)], o_rest_sem)

    def fetch(h, slot):
        copy_q(h, slot).start()
        copy_k(h, slot).start()
        copy_v(h, slot).start()

    def block(h0, n, zero, emit):
        prev_lane_sum = None
        for j in range(n):
            h = h0 + j
            copy_q(h, j).wait()
            copy_k(h, j).wait()
            s = lax.dot_general(q_buf[j], k_buf[j], (((1,), (1,)), ((), ())),
                                preferred_element_type=jnp.float32)

            @pl.when(h + prefetch < n_heads)
            def _(h=h, j=j):
                fetch(h + prefetch, (j + prefetch) % group)

            if prev_lane_sum is None:
                scale = c
            else:
                scale = jnp.concatenate(
                    [jnp.where(prev_lane_sum >= 0.0, c, c + zero)] * n_tiles, axis=-1)

            m = jnp.max(s, axis=-1, keepdims=True)
            p = jnp.exp2((s - m) * scale)
            lane_sum = p[:, :_LANES]
            for t in range(1, n_tiles):
                lane_sum = lane_sum + p[:, t * _LANES:(t + 1) * _LANES]
            prev_lane_sum = lane_sum

            copy_v(h, j).wait()
            o = jnp.dot(p.astype(v_buf.dtype), v_buf[j], preferred_element_type=jnp.float32)
            l = jnp.sum(lane_sum, axis=-1, keepdims=True)
            emit(j, (o * pl.reciprocal(l, approx=True)).astype(o_buf.dtype))

    def main_block(it, carry):
        h0 = it * group

        def emit(j, out):
            if j in piece_of_first:
                @pl.when(it > 0)
                def _():
                    copy_o(h0 - group, piece_of_first[j]).wait()
            o_buf[j] = out
            if j in piece_of_last:
                copy_o(h0, piece_of_last[j]).start()

        zero = jnp.minimum(it, 0).astype(jnp.float32)
        block(h0, group, zero, emit)
        return carry

    for j in range(prefetch):
        fetch(j, j)
    lax.fori_loop(0, n_main // group, main_block, 0)

    if rest:
        def emit_rest(j, out):
            o_rest_buf[j] = out
            if j == rest - 1:
                copy_o_rest().start()

        block(n_main, rest, jnp.minimum(pl.program_id(0), 0).astype(jnp.float32), emit_rest)

    for piece in range(len(pieces)):
        copy_o(n_main - group, piece).wait()
    if rest:
        copy_o_rest().wait()


@jax.jit
def pallas_standalone__mha_softmax__near_ridge_kernel(q: jax.Array, k: jax.Array, v: jax.Array):
    b, h, sq, d = q.shape
    sk = k.shape[2]
    n_heads = b * h
    assert sk % _LANES == 0, k.shape
    group, rest = _split_heads(n_heads)
    prefetch = min(_MAX_PREFETCH, group - 1)
    pieces = _pieces(group, min(_MAX_OUT_PIECES, group))

    out = pl.pallas_call(
        functools.partial(_attention_kernel, rest=rest, prefetch=prefetch, pieces=pieces),
        grid=(1,),
        in_specs=[pl.BlockSpec(memory_space=pl.ANY)] * 3,
        out_specs=pl.BlockSpec(memory_space=pl.ANY),
        out_shape=jax.ShapeDtypeStruct((n_heads, sq, d), q.dtype),
        scratch_shapes=[
            pltpu.VMEM((group, sq, d), q.dtype),
            pltpu.VMEM((group, sk, d), k.dtype),
            pltpu.VMEM((group, sk, d), v.dtype),
            pltpu.VMEM((group, sq, d), q.dtype),
            pltpu.VMEM((max(rest, 1), sq, d), q.dtype),
            pltpu.SemaphoreType.DMA((group,)),
            pltpu.SemaphoreType.DMA((group,)),
            pltpu.SemaphoreType.DMA((group,)),
            pltpu.SemaphoreType.DMA((len(pieces),)),
            pltpu.SemaphoreType.DMA(()),
        ],
        compiler_params=pltpu.CompilerParams(
            dimension_semantics=("arbitrary",),
            vmem_limit_bytes=96 << 20,
            flags={"XLA_TPU_RESCHEDULE_DMA_DONES": True},
            disable_bounds_checks=True,
            disable_semaphore_checks=True,
        ),
    )(q.reshape(n_heads, sq, d), k.reshape(n_heads, sk, d), v.reshape(n_heads, sk, d))
    return out.reshape(q.shape)
```
